```python
import os as _os
_os.environ.setdefault("JAX_PLATFORMS", "cpu")
import jax
import jax.numpy as jnp

def _softmax(x, axis=-1):
    return jax.nn.softmax(x, axis=axis)
def _gelu(x):
    return jax.nn.gelu(x, approximate=True)
def _silu(x):
    return jax.nn.silu(x)
def _sigmoid(x):
    return jax.nn.sigmoid(x)
def _layernorm(x, axis=-1, eps=1e-5):
    m = jnp.mean(x, axis=axis, keepdims=True)
    v = jnp.var(x, axis=axis, keepdims=True)
    return (x - m) / jnp.sqrt(v + eps)
def _scatter_add(tgt, idx, src, axis=0):
    return tgt.at[idx].add(src)
def _segment_sum(src, seg, n):
    return jax.ops.segment_sum(src, seg, n)
class _Rng:
    def __init__(self, key):
        self._k = key
    def _next(self):
        self._k, sub = jax.random.split(self._k)
        return sub
    def normal(self, shape):
        return jax.random.normal(self._next(), shape, dtype=jnp.bfloat16)
    def randint(self, lo, hi, shape):
        return jax.random.randint(self._next(), shape, lo, hi, dtype=jnp.int32)
    def uniform(self, shape, lo=0.0, hi=1.0):
        return jax.random.uniform(self._next(), shape, jnp.bfloat16, lo, hi)
    def permutation(self, n):
        return jax.random.permutation(self._next(), n)


kernel_name = 'recurrent_scan__ssm_conv_s5__geglu_ffn__prompt'

def setup_inputs():
    _rng = _Rng(jax.random.key(int.from_bytes(__import__("os").urandom(4), "little")))
    _w = (lambda a: (lambda t: t.astype(jnp.bfloat16) if jnp.issubdtype(t.dtype, jnp.floating) else t)(jnp.asarray(a)))
    def _A_setup():
        B, S, D = 1, 2048, 640
        P = D
        Lambda_re = -0.5 * jnp.exp((lambda *s: _rng.normal(s) * 0.4)(P))
        Lambda_im = (lambda *s: _rng.normal(s) * 0.4)(P) * 1.0
        B_re = (lambda *s: _rng.normal(s) * 0.4)(P, D) * (D ** -0.5)
        B_im = (lambda *s: _rng.normal(s) * 0.4)(P, D) * (D ** -0.5)
        C_re = (lambda *s: _rng.normal(s) * 0.4)(D, P) * (P ** -0.5)
        C_im = (lambda *s: _rng.normal(s) * 0.4)(D, P) * (P ** -0.5)
        log_dt = (lambda *s: _rng.normal(s) * 0.4)(P) * 0.3 - 2.0
        Dskip = (lambda *s: _rng.normal(s) * 0.4)(D)
        return {
            "x": _w((lambda *s: _rng.normal(s) * 0.05)(B, S, D)),
            "Lambda_re": _w(Lambda_re),
            "Lambda_im": _w(Lambda_im),
            "B_re": _w(B_re),
            "B_im": _w(B_im),
            "C_re": _w(C_re),
            "C_im": _w(C_im),
            "log_dt": _w(log_dt),
            "Dskip": _w(Dskip),
        }
    _A_in = _A_setup()

    def _B_setup():
        B, S, D, F = 1, 2048, 640, 1728
        return {
            "x": _w((lambda *s: _rng.normal(s) * 0.05)(B, S, D)),
            "w_gate": _w((lambda *s: _rng.normal(s) * 0.05)(D, F)),
            "w_up": _w((lambda *s: _rng.normal(s) * 0.05)(D, F)),
            "w_down": _w((lambda *s: _rng.normal(s) * 0.05)(F, D)),
        }
    _B_in = _B_setup()

    return {
        "A_x": _A_in["x"],
        "A_Lambda_re": _A_in["Lambda_re"],
        "A_Lambda_im": _A_in["Lambda_im"],
        "A_B_re": _A_in["B_re"],
        "A_B_im": _A_in["B_im"],
        "A_C_re": _A_in["C_re"],
        "A_C_im": _A_in["C_im"],
        "A_log_dt": _A_in["log_dt"],
        "A_Dskip": _A_in["Dskip"],
        "B_x": _B_in["x"],
        "B_w_gate": _B_in["w_gate"],
        "B_w_up": _B_in["w_up"],
        "B_w_down": _B_in["w_down"],
    }

def reference(A_x, A_Lambda_re, A_Lambda_im, A_B_re, A_B_im, A_C_re, A_C_im, A_log_dt, A_Dskip, B_x, B_w_gate, B_w_up, B_w_down):
    def _A_ref(x, Lambda_re, Lambda_im, B_re, B_im, C_re, C_im, log_dt, Dskip):
        Bsz, L, H = x.shape
        Lam = Lambda_re + 1j * Lambda_im
        Bmat = B_re + 1j * B_im
        Cmat = C_re + 1j * C_im
        dt = jnp.exp(log_dt)
        Lam_bar = jnp.exp(dt * Lam)
        B_bar = ((Lam_bar - 1.0) / Lam)[:, None] * Bmat
        Bu = jnp.einsum("bld,pd->blp", x + 0j, B_bar)
        h = jnp.zeros_like(Bu[:, 0, :])
        hs = []
        for t in range(L):
            h = Lam_bar[None, :] * h + Bu[:, t, :]
            hs.append(h)
        hseq = jnp.stack(hs, 1)
        y = 2.0 * jnp.einsum("blp,dp->bld", hseq, Cmat).real + x * Dskip[None, None, :]
        return y

    def _B_ref(x, w_gate, w_up, w_down):
        return (_gelu(x @ w_gate) * (x @ w_up)) @ w_down

    x = A_x
    xn = _layernorm(x, axis=-1)
    s = _A_ref(xn, A_Lambda_re, A_Lambda_im, A_B_re, A_B_im, A_C_re, A_C_im, A_log_dt, A_Dskip)
    g = _silu(_B_ref(xn, B_w_gate, B_w_up, B_w_down))
    return x + s * g
```

```python
import jax
import jax.numpy as jnp
from jax import lax
import jax.experimental.pallas as pl
import jax.experimental.pallas.tpu as pltpu

f32, bf16, u32 = jnp.float32, jnp.bfloat16, jnp.uint32

L, D, P, F = 2048, 640, 640, 1728
T = 256
R = T // 2
NB = L // T
CH = R // 8
CS = CH + 1
HR = (8 * CS + CH + 7) // 8 * 8
RS = 64
RT = 32


def _parse(rows):
    def form(text):
        terms = {}
        for term in text.split():
            sign = term[:-2]
            terms[int(term[-2]), int(term[-1])] = len(sign) * (1 if sign[0] == "+" else -1)
        return terms
    return [tuple(form(part) for part in row.split("|")) for row in rows]


K5 = _parse([
    "+00 +10 | +00 -01 -04 +14 -20 | +10",
    "+00 | +00 -02 -10 -40 +41 | +00 -10",
    "+01 +11 | +03 -10 +11 -13 -21 | +01",
    "+11 | +01 -11 +12 -30 +31 | +01 -11",
    "+02 | -12 -20 +22 -23 -42 | +02",
    "+12 | -02 -21 +22 -24 -32 | +12",
    "+03 +13 | -03 -23 +30 -31 +33 -34 | +13",
    "+03 | +03 -13 -30 -32 +33 -43 | +03 -13",
    "+04 +14 | -14 -24 -40 +41 -43 +44 | +04",
    "+14 | +04 -14 +34 +41 +42 -44 | +04 -14",
    "+00 +01 | -03 +10 -41 | +00 +01",
    "+10 +11 | +01 -14 -30 | +10 +11",
    "+00 -11 | +01 -10 | +01 +10",
    "+00 +02 +10 +12 | +20 | +00 +02",
    "+10 +12 | -02 | +00 +02 -10 -12",
    "+00 +10 +12 | +02 -20 | +00 +02 -10",
    "+00 +01 +03 +10 +11 +13 | +03 | +00 +01 +03",
    "+10 +11 +13 | -30 | +00 +01 +03 -10 -11 -13",
    "+03 +10 +11 +13 | -03 +30 | +00 +01 +03 -13",
    "+00 +04 | +40 -41 | +00 +04",
    "+10 +14 | +04 -14 | +10 +14",
    "+00 -14 | +04 -14 -40 +41 | +04 +10",
    "+01 +02 +11 +12 | +21 | +11 +12",
    "+01 +02 | +12 | +01 +02 -11 -12",
    "+01 +02 +11 | -12 +21 | +01 -11 -12",
    "+01 +03 | -03 +13 | +01 +03",
    "+11 +13 | -30 +31 | +11 +13",
    "-03 +11 | -03 +13 +30 -31 | +01 +13",
    "+00 +01 +04 +10 +11 +14 | +14 | +10 +11 +14",
    "+00 +01 +04 | +41 | +00 +01 +04 -10 -11 -14",
    "+00 +01 +04 +14 | -14 +41 | -04 +10 +11 +14",
    "+02 +03 +12 +13 | +23 | +02 +03",
    "+12 +13 | -32 | +02 +03 -12 -13",
    "+03 +12 +13 | -23 +32 | +02 +03 -13",
    "+02 +04 +12 +14 | +24 | +12 +14",
    "+02 +04 | +42 | +02 +04 -12 -14",
    "+02 +04 +14 | -24 +42 | -04 +12 +14",
    "+03 +04 | +43 | +03 +04",
    "+13 +14 | +34 | +13 +14",
    "+03 -14 | +34 -43 | +04 +13",
])
K5_ROUNDS = [[13, 14, 15, 4], [22, 23, 24, 5], [34, 35, 36, 8], [31, 32, 33, 6], [37, 38, 39, 7], [25, 26, 27, 2], [16, 17, 18, 0], [19, 20, 21, 9], [28, 29, 30, 3], [10, 11, 12, 1]]

N2 = _parse([
    "+00 +10 | +00 -01 | +10",
    "+00 | +00 -10 | +00 -10",
    "+01 +11 | -10 +11 | +01",
    "+11 | +01 -11 | +01 -11",
    "+00 +01 | +10 | +00 +01",
    "+10 +11 | +01 | +10 +11",
    "+00 -11 | +01 -10 | +01 +10",
    "+03 +13 | +30 -31 | +10",
    "+03 | +30 -40 | +00 -10",
    "+04 +14 | -40 +41 | +01",
    "+14 | +31 -41 | +01 -11",
    "+03 +04 | +40 | +00 +01",
    "+13 +14 | +31 | +10 +11",
    "+03 -14 | +31 -40 | +01 +10",
    "+02 | +20 | +00",
    "+12 | +20 | +10",
    "+02 | +21 | +01",
    "+12 | +21 | +11",
])
N2_ROUNDS = [[0, 1, 2, 3], [4, 5, 6, 7], [8, 9, 10, 11], [12, 13, 14, 15], [16, 17]]

K7 = _parse([
    "+00 +10 | -00 +02 +03 +24 -51 | +10",
    "+00 | -01 -02 +03 -04 -13 | +00 -10",
    "+01 +11 | +10 -12 +14 -20 | +01",
    "+11 | +00 -02 -10 +11 --13 -14 +30 +60 -62 | +01 -11",
    "+02 | -11 +13 +21 -22 ++24 -41 | +02",
    "+12 | -01 +03 -20 +21 -23 -31 | +12",
    "+03 +13 | -22 -30 +32 -33 +50 -52 | +13",
    "+03 | -12 -13 -14 -31 +32 -34 +40 -42 | +03 -13",
    "+04 +14 | -23 -24 -42 +43 +51 -53 | +04",
    "+14 | +33 +40 +41 -43 +44 -61 +63 | +04 -14",
    "+05 | +02 -40 -44 +50 -52 +54 | +05",
    "+15 | -02 -03 -04 -34 +50 ++51 -53 +54 -62 -64 | +15",
    "+06 +16 | +02 -50 -60 ++62 -63 | +16",
    "+06 | -02 +13 +14 -40 -64 | +06 -16",
    "+00 +01 | +13 | +00 +01",
    "+10 +11 | +00 -02 | +10 +11",
    "+00 -11 | +00 -02 -13 | +01 +10",
    "+00 +02 +10 +12 | -24 | +00 +02",
    "+10 +12 | -01 +03 | +00 +02 -10 -12",
    "+00 +10 +12 | +01 -03 +24 | +00 +02 -10",
    "+01 +02 +11 +12 | +20 | +11 +12",
    "+01 +02 | +11 -13 | +01 +02 -11 -12",
    "+01 +02 +11 | -11 +13 +20 | +01 -11 -12",
    "+01 +03 | +12 +13 +14 | +01 +03",
    "+11 +13 | +30 | +11 +13",
    "-03 +11 | +12 +13 +14 -30 | +01 +13",
    "+02 +03 +12 +13 | +22 | +02 +03",
    "+12 +13 | -31 | +02 +03 -12 -13",
    "+03 +12 +13 | -22 +31 | +02 +03 -13",
    "+02 +04 +12 +14 | +23 +24 | +12 +14",
    "+02 +04 | +41 | +02 +04 -12 -14",
    "+02 +04 +14 | -23 -24 +41 | -04 +12 +14",
    "+03 +04 | -40 +42 | +03 +04",
    "+13 +14 | +33 | +13 +14",
    "+03 -14 | +33 +40 -42 | +04 +13",
    "+03 +05 +13 +15 | -50 +52 | +03 +05",
    "+13 +15 | -34 | +03 +05 -13 -15",
    "+03 +13 +15 | +34 +50 -52 | +03 +05 -13",
    "+04 +05 +14 +15 | -51 +53 | +14 +15",
    "+04 +05 | +40 +44 | +04 +05 -14 -15",
    "+04 +05 +14 | -40 -44 -51 +53 | +04 -14 -15",
    "+04 +06 | +40 | +04 +06",
    "+14 +16 | -61 +63 | +14 +16",
    "-06 +14 | +40 +61 -63 | +04 +16",
    "+05 +06 +15 +16 | -02 +50 | +05 +06",
    "+15 +16 | -62 -64 | +05 +06 -15 -16",
    "+06 +15 +16 | +02 -50 +62 +64 | +05 +06 -16",
    "+00 +05 +10 +15 | -02 +51 | +00 +05",
    "+10 +15 | -02 -03 -04 +61 | +00 +05 -10 -15",
    "+00 +10 +15 | +02 +03 +04 -51 | +00 +05 -10",
    "+00 +05 +06 | +02 | +00 +05 +06",
    "+10 +15 +16 | +61 | +10 +15 +16",
    "-06 +10 +15 | +02 -61 | +00 +05 +16",
    "+01 +06 | -13 -14 | +01 +06",
    "+11 +16 | +60 -62 | +11 +16",
    "+06 -11 | +13 +14 +60 -62 | +01 +16",
])
K7_ROUNDS = [[41, 42, 43, 12], [44, 45, 46, 13], [47, 48, 49, 0], [50, 51, 52, 1], [53, 54, 55, 2], [14, 15, 16, 3], [17, 18, 19, 4], [20, 21, 22, 5], [23, 24, 25, 6], [26, 27, 28, 7], [38, 39, 40, 10], [32, 33, 34, 8], [35, 36, 37, 11], [29, 30, 31, 9]]
K7_FOLD = {6: {0: 1, 2: 1, 4: -1}, 0: {1: 1, 3: 1, 4: -1}}


def _key(form):
    return tuple(sorted(form.items()))


X_SLOT = {_key(u): r for r, (u, _, _) in enumerate(K5)}

K5_TILES = [(4, 1), (4, 0), (2, 0), (0, 4), (3, 0), (0, 1), (1, 4), (0, 0), (1, 0), (0, 2), (3, 1), (1, 3), (0, 3),
            (1, 1), (1, 2), (2, 1), (2, 2), (2, 4), (3, 2), (2, 3), (4, 2), (3, 4), (3, 3), (4, 3), (4, 4)]
K7_TILES = [(6, 0), (6, 3), (5, 0), (6, 2), (0, 2), (6, 4), (0, 4), (3, 4), (6, 1), (0, 3), (5, 2), (5, 1),
            (5, 3), (5, 4), (4, 0), (4, 4), (2, 4), (0, 0), (0, 1), (1, 3), (1, 4), (1, 0), (1, 1), (1, 2),
            (2, 0), (2, 1), (3, 0), (2, 2), (2, 3), (3, 1), (4, 2), (3, 2), (3, 3), (4, 1), (4, 3)]
N2_TILES = [(k, q) for k in range(5) for q in range(2)]

GROUPS = {
    "bre": (K5, K5_TILES, True), "bim": (K5, K5_TILES, True),
    "gA": (K5, K5_TILES, True), "uA": (K5, K5_TILES, True),
    "gB": (K5, K5_TILES, True), "uB": (K5, K5_TILES, True),
    "m": (K5, K5_TILES, True), "l": (N2, N2_TILES, True),
    "dA": (K7, K7_TILES, False), "dB": (K7, K7_TILES, False),
    "cre": (K5, K5_TILES, True), "cim": (K5, K5_TILES, True),
}
W_BASE = {}
NW = 0
for _name, (_scheme, _tiles, _flag) in GROUPS.items():
    W_BASE[_name] = NW
    NW += len(_scheme)


def _signed_sums(forms, get):
    forms = [dict(form) for form in forms]
    values = {}

    def value(k):
        if k not in values:
            values[k] = get(k)
        return values[k]

    n = 0
    while True:
        count = {}
        for form in forms:
            keys = sorted(form, key=repr)
            for i in range(len(keys)):
                for j in range(i + 1, len(keys)):
                    pair = (keys[i], keys[j], form[keys[i]] * form[keys[j]])
                    count[pair] = count.get(pair, 0) + 1
        if not count:
            break
        (a, b, sign), _ = max(count.items(), key=lambda kv: kv[1])
        t = ("t", n)
        n += 1
        values[t] = value(a) + value(b) if sign > 0 else value(a) - value(b)
        for form in forms:
            if a in form and b in form and form[a] * form[b] == sign:
                form[t] = form[a]
                del form[a], form[b]
    result = []
    for form in forms:
        (k, sign), = form.items()
        result.append((sign, value(k)))
    return result


class _Symbol:
    def __init__(self, name, program):
        self.name, self.program = name, program

    def _combine(self, other, sign):
        t = _Symbol(("t", len(self.program)), self.program)
        self.program.append((t.name, self.name, other.name, sign))
        return t

    def __add__(self, other):
        return self._combine(other, 1)

    def __sub__(self, other):
        return self._combine(other, -1)


def _sum_program(forms):
    program = []
    outs = _signed_sums(forms, lambda k: _Symbol(k, program))
    return program, [(sign, v.name) for sign, v in outs]


def _accumulate(acc, outs, products):
    keys = sorted(set(k for w in outs for k in w))
    forms = [{i: w[k] * products[i][0] for i, w in enumerate(outs) if k in w} for k in keys]
    for k, (sign, v) in zip(keys, _signed_sums(forms, lambda i: products[i][1])):
        if k not in acc:
            acc[k] = (sign, v)
        else:
            sign0, a = acc[k]
            if sign0 == sign:
                acc[k] = (sign0, a + v)
            elif sign0 > 0:
                acc[k] = (1, a - v)
            else:
                acc[k] = (1, v - a)


def _finish(acc):
    return {k: (v if sign > 0 else -v) for k, (sign, v) in acc.items()}


def _cmul(ar, ai, br, bi):
    return ar * br - ai * bi, ar * bi + ai * br


def _geglu2(g, u):
    inner = g * (0.7978845608028654 + 0.7978845608028654 * 0.044715 * (g * g))
    p = g * u
    return p + p * jnp.tanh(inner)


def _drain(gen):
    for _ in gen:
        pass


def _chain(*gens):
    for gen in gens:
        yield from gen


def _take(gen, n):
    for _ in range(n):
        if next(gen, StopIteration) is StopIteration:
            return
        yield


def _merge(fg, n_fg, bg, n_bg, upto=1.0, since=0.0):
    lo = int(n_fg * since)
    hi = max(lo + 1, int(n_fg * upto))
    done = i = 0
    for _ in fg:
        i += 1
        if i > lo:
            want = min(n_bg, (i - lo - 1) * n_bg // (hi - lo) + 1)
            while done < want:
                if next(bg, StopIteration) is StopIteration:
                    done = n_bg
                    break
                done += 1
        yield
    _drain(bg)


def _kernel(x_hbm, lre_hbm, lim_hbm, bre_hbm, bim_hbm, cre_hbm, cim_hbm, ldt_hbm, dsk_hbm,
            wg_hbm, wu_hbm, wd_hbm, o_hbm,
            x_s, bre_s, bim_s, cre_s, cim_s, wg_s, wu_s, wd_s,
            w_s, xc_s, st_s, xn_s, par_s, carry_s, bu_s, h_s, a_s, y_s, z_s, o_s,
            lre_s, lim_s, ldt_s, dsk_s, in_sem, out_sem, zero_sem):
    x_copy = [pltpu.make_async_copy(x_hbm.at[pl.ds(b * T, T)], x_s.at[pl.ds(b * T, T)], in_sem.at[b])
              for b in range(NB)]
    copy = {}
    pieces = [("bre", bre_hbm, bre_s, 0, P), ("bim", bim_hbm, bim_s, 0, P)]
    for tag, lo, hi in [("A", 0, 640), ("B", 640, 1280), ("m", 1280, 1600), ("l", 1600, F)]:
        pieces += [("g" + tag, wg_hbm, wg_s, lo, hi), ("u" + tag, wu_hbm, wu_s, lo, hi)]
    pieces += [("dA", wd_hbm, wd_s, 0, 896), ("dB", wd_hbm, wd_s, 896, F),
               ("cre", cre_hbm, cre_s, 0, D), ("cim", cim_hbm, cim_s, 0, D)]
    for i, (name, src, dst, lo, hi) in enumerate(pieces):
        copy[name] = pltpu.make_async_copy(src.at[pl.ds(lo, hi - lo)], dst.at[pl.ds(lo, hi - lo)],
                                           in_sem.at[NB + i])
    small = [pltpu.make_async_copy(src, dst, in_sem.at[NB + len(pieces) + i]) for i, (src, dst) in
             enumerate([(lre_hbm, lre_s), (lim_hbm, lim_s), (ldt_hbm, ldt_s), (dsk_hbm, dsk_s)])]
    for cp in small + x_copy[:2]:
        cp.start()
    for name in ("gl", "ul", "bre", "bim", "gA", "uA", "gB", "uB", "gm", "um", "cre", "cim", "dA", "dB"):
        copy[name].start()
    for cp in x_copy[2:]:
        cp.start()

    keep = lax.broadcasted_iota(jnp.int32, (8, 128), 0) >= pl.semaphore_read(zero_sem)
    latest = [None]
    now = [0]
    due = []

    def after(v):
        return v if latest[0] is None else jnp.where(keep, v, latest[0])

    def before(v, slack):
        if latest[0] is not None:
            due.append((now[0] + slack, v))

    def gate(lhs, span):
        n = lhs.shape[0] // 8
        for i, (t, v) in enumerate(due):
            if t < now[0] + span:
                j = min(n - 1, max(0, (t - now[0]) * n // span))
                parts = [lhs[k * 8:(k + 1) * 8] for k in range(n)]
                if v.dtype != lhs.dtype:
                    v = lax.bitcast_convert_type(v, lhs.dtype)
                parts[j] = jnp.where(keep, parts[j], v)
                del due[i]
                return jnp.concatenate(parts, axis=0)
        return lhs

    def results(products, rows):
        for j in range(rows // 8):
            latest[0] = products[j % len(products)][1][j * 8:(j + 1) * 8]
            now[0] += 1
            yield

    def reset():
        latest[0] = None
        due.clear()

    def wait(*names):
        for name in names:
            copy[name].wait()
        reset()

    def ssm_params():
        for cp in small:
            cp.wait()
        lre = lre_s[...].astype(f32).reshape(1, P)
        lim = lim_s[...].astype(f32).reshape(1, P)
        dt = jnp.exp(ldt_s[...].astype(f32).reshape(1, P)).astype(bf16).astype(f32)
        mag = jnp.exp(dt * lre)
        ar = mag * jnp.cos(dt * lim)
        ai = mag * jnp.sin(dt * lim)
        s = jnp.maximum(jnp.abs(lre), jnp.abs(lim))
        cr, ci = lre / s, lim / s
        den = (cr * cr + ci * ci) * s
        nr, ni = ar - 1.0, ai
        kr = 2.0 * (nr * cr + ni * ci) / den
        ki = 2.0 * (ni * cr - nr * ci) / den
        pr, pi = ar, ai
        n = 1
        while n < CH:
            pr, pi = _cmul(pr, pi, pr, pi)
            n *= 2
        values = [ar, ai, kr, ki, pr, pi]
        for _ in range(2):
            pr, pi = _cmul(pr, pi, pr, pi)
            values += [pr, pi]
        values.append(dsk_s[...].astype(f32).reshape(1, D))
        for i, v in enumerate(values):
            for c in range(5):
                par_s[i, c] = jnp.broadcast_to(v[:, c * 128:(c + 1) * 128], (8, 128))
        carry_s[...] = jnp.zeros_like(carry_s)

    x_sign = {}

    def first_row(b):
        return b * T if isinstance(b, int) else pl.multiple_of(b * T, T)

    def normalise(x16, e):
        xs = [x16[e * 8:e * 8 + 8, c * 128:(c + 1) * 128] for c in range(5)]
        xs[0] = after(xs[0])
        mu = jnp.sum((xs[0] + xs[1]) + (xs[2] + xs[3]) + xs[4], axis=-1, keepdims=True) * (1.0 / D)
        xs = [v - mu for v in xs]
        sq = [v * v for v in xs]
        var = jnp.sum((sq[0] + sq[1]) + (sq[2] + sq[3]) + sq[4], axis=-1, keepdims=True) * (1.0 / D)
        return xs, mu, lax.rsqrt(var + 1e-5)

    def save_stats(slot, row, mu, rstd):
        st_s[slot * 2, pl.ds(row, 8), :] = jnp.broadcast_to(mu, (8, 128))
        st_s[slot * 2 + 1, pl.ds(row, 8), :] = jnp.broadcast_to(rstd, (8, 128))

    def norm_and_sums(b, slot):
        order = [r for rnd in K5_ROUNDS for r in rnd]
        for i in range(R // 16):
            xn = {}
            for m in range(2):
                x16 = x_s[pl.ds(b * T + m * R + i * 16, 16), :].astype(f32)
                for e in range(2):
                    xs, mu, rstd = normalise(x16, e)
                    for c in range(5):
                        xn[e, m, c] = xs[c] * rstd
                    save_stats(b, m * R + i * 16 + e * 8, mu, rstd)
            sums = [_signed_sums([K5[r][0] for r in order], lambda mc: xn[e, mc[0], mc[1]]) for e in range(2)]
            for j, r in enumerate(order):
                x_sign[r] = sums[0][j][0]
                xc_s[slot, r, pl.ds(i * 16, 16), :] = jnp.concatenate(
                    [sums[0][j][1], sums[1][j][1]], axis=0).astype(bf16)

    def stage_norm(b, stat_slot):
        row0 = first_row(b)
        for i in range(T // 16):
            x16 = x_s[pl.ds(row0 + i * 16, 16), :].astype(f32)
            for e in range(2):
                xs, mu, rstd = normalise(x16, e)
                for c in range(5):
                    v = xs[c] * rstd
                    xn_s[c, pl.ds(i * 16 + e * 8, 8), :] = v
                save_stats(stat_slot, i * 16 + e * 8, mu, rstd)
                before(v, 64)
                yield
    n_norm = T // 8

    def stage_sums():
        for i in range(R // 16):
            for rnd in K5_ROUNDS:
                loaded = {}

                def get(mc):
                    if mc not in loaded:
                        v = xn_s[mc[1], pl.ds(mc[0] * R + i * 16, 16), :]
                        loaded[mc] = v if loaded else jnp.concatenate([after(v[:8]), after(v[8:])], axis=0)
                    return loaded[mc]

                for r, (sign, v) in zip(rnd, _signed_sums([K5[r][0] for r in rnd], get)):
                    xc_s[0, r, pl.ds(i * 16, 16), :] = (v if sign == x_sign[r] else -v).astype(bf16)
                before(v[8:], 28)
                yield
    n_sums = (R // 16) * len(K5_ROUNDS)

    def rows16(ref, row, col):
        return ref[pl.ds(row, 16), pl.ds(col, 128)]

    def tiles_nk(ref, row0):
        return lambda k, q, i: rows16(ref, row0 + q * 128 + i, k * 128)

    def tiles_mixed(k, q, i):
        return rows16(wg_s if i < 64 else wu_s, 1280 + q * 64 + i % 64, k * 128)

    def tiles_last(k, q, i):
        return rows16(wg_s if q == 0 else wu_s, 1600 + i, k * 128)

    def tiles_down_a(k, q, i):
        return rows16(wd_s, k * 128 + i, q * 128)

    def tiles_down_b(k, q, i):
        if k == 5 and i >= 64:
            return jnp.zeros((16, 128), bf16)
        return rows16(wd_s, (896 + k * 128 if k < 6 else 1600) + i, q * 128)

    tiles = {"bre": tiles_nk(bre_s, 0), "bim": tiles_nk(bim_s, 0),
             "gA": tiles_nk(wg_s, 0), "uA": tiles_nk(wu_s, 0),
             "gB": tiles_nk(wg_s, 640), "uB": tiles_nk(wu_s, 640),
             "m": tiles_mixed, "l": tiles_last, "dA": tiles_down_a, "dB": tiles_down_b,
             "cre": tiles_nk(cre_s, 0), "cim": tiles_nk(cim_s, 0)}
    w_sign = {}
    ready = []

    def prepare(name):
        scheme, need, _ = GROUPS[name]
        base = W_BASE[name]
        forms = [{(k if abs(c) == 1 else k + (abs(c),)): (1 if c > 0 else -1) for k, c in v.items()}
                 for _, v, _ in scheme]
        program, outs = _sum_program(forms)
        for i in range(0, 128, 16):
            val, todo, left = {}, list(program), list(range(len(scheme)))
            for kq in need:
                w = tiles[name](*kq, i).astype(f32)
                val[kq] = [after(w[:8]), w[8:]]
                for k in sorted(set(k for form in forms for k in form if len(k) == 3 and k[:2] == kq)):
                    val[k] = [v * float(k[2]) for v in val[kq]]
                for step in list(todo):
                    t, a, b, sign = step
                    if a in val and b in val:
                        val[t] = [val[a][e] + val[b][e] if sign > 0 else val[a][e] - val[b][e] for e in range(2)]
                        todo.remove(step)
                for r in list(left):
                    if outs[r][1] in val:
                        w_sign[base + r] = outs[r][0]
                        w_s[base + r, pl.ds(i, 16), :] = jnp.concatenate(val[outs[r][1]], axis=0).astype(bf16)
                        left.remove(r)
                if i == 112 and kq == need[-1]:
                    assert not left
                    ready.append(name)
                yield

    def prepares(*names):
        return _chain(*[prepare(name) for name in names]), sum(8 * len(GROUPS[name][1]) for name in names)

    w_words, xc_words = w_s.bitcast(u32), xc_s.bitcast(u32)

    def product(lhs, name, r):
        assert name in ready
        dims = (((1,), (1,)), ((), ())) if GROUPS[name][2] else (((1,), (0,)), ((), ()))
        rhs = pltpu.bitcast(w_words[W_BASE[name] + r], bf16)
        return lax.dot_general(lhs, rhs, dims, preferred_element_type=f32)

    def in_product(result, slot, name):
        scheme = GROUPS[name][0]
        acc = {}
        for rnd in (N2_ROUNDS if name == "l" else K5_ROUNDS):
            products = []
            for r in rnd:
                xr = X_SLOT[_key(scheme[r][0])]
                lhs = pltpu.bitcast(gate(xc_words[slot, xr], R // 8), bf16)
                products.append((x_sign[xr] * w_sign[W_BASE[name] + r], product(lhs, name, r)))
            _accumulate(acc, [scheme[r][2] for r in rnd], products)
            yield from results(products, R)
        result.update(_finish(acc))
    n_group = (R // 8) * len(K5_ROUNDS)

    def state_row(slot, part, m, c):
        return ((slot * 2 + part) * 2 + m) * 5 + c

    def stage_b(slot, part):
        bu = {}
        yield from in_product(bu, slot, ("bre", "bim")[part])
        for (m, q), v in bu.items():
            for k in range(8):
                bu_s[state_row(slot, part, m, q), pl.ds(k * CS, CH), :] = v[k * CH:(k + 1) * CH]

    def stage_up(gates, slot, group):
        up = {}
        yield from in_product(up, slot, "u" + "AB"[group])
        for m, q in up:
            a_s[slot, group * 5 + q, m] = _geglu2(gates[m, q], up[m, q])

    def stage_ffn(slot, group):
        gates = {}
        yield from in_product(gates, slot, "g" + "AB"[group])
        yield from stage_up(gates, slot, group)

    def stage_mixed(slot):
        low = lax.broadcasted_iota(jnp.int32, (R, 128), 1) < 64
        t = {}
        yield from in_product(t, slot, "m")
        for m in range(2):
            for i in range(2):
                t1, t2 = t[m, 2 * i], t[m, 2 * i + 1]
                g = jnp.where(low, t1, pltpu.roll(t2, 64, 1))
                u = jnp.where(low, pltpu.roll(t1, 64, 1), t2)
                a_s[slot, 10 + i, m] = _geglu2(g, u)
            a_s[slot, 12, m] = jnp.where(low, _geglu2(t[m, 4], pltpu.roll(t[m, 4], 64, 1)), 0.0)

    def stage_last(slot):
        t = {}
        yield from in_product(t, slot, "l")
        for m in range(2):
            a_s[slot, 13, m] = _geglu2(t[m, 0], t[m, 1])
    n_ffn = 5 * n_group + (R // 8) * len(N2_ROUNDS)

    def stage_scan(slot, slack):
        row = lax.broadcasted_iota(jnp.int32, (8, 128), 0)

        def step(m, c, j, ar, ai, hr, hi):
            tr, ti = _cmul(ar, ai, hr, hi)
            return tr + bu(0, m, c, j), ti + bu(1, m, c, j)

        def bu(part, m, c, j):
            return bu_s[state_row(slot, part, m, c), pl.ds(j, 8, stride=CS), :]

        for c in range(5):
            in_r, in_i = carry_s[0, c], carry_s[1, c]
            for m in range(2):
                ar, ai = par_s[0, c], par_s[1, c]
                kr, ki = par_s[2, c], par_s[3, c]
                hr, hi = after(bu(0, m, c, 0)), after(bu(1, m, c, 0))
                for j in range(1, CH):
                    hr, hi = step(m, c, j, ar, ai, hr, hi)
                tr, ti = _cmul(par_s[4, c], par_s[5, c], in_r, in_i)
                er = hr + jnp.where(row == 0, tr, 0.0)
                ei = hi + jnp.where(row == 0, ti, 0.0)
                for level, d in enumerate((1, 2, 4)):
                    sr = jnp.where(row >= d, pltpu.roll(er, d, 0), 0.0)
                    si = jnp.where(row >= d, pltpu.roll(ei, d, 0), 0.0)
                    tr, ti = _cmul(par_s[4 + 2 * level, c], par_s[5 + 2 * level, c], sr, si)
                    er, ei = er + tr, ei + ti
                hr = jnp.where(row == 0, in_r, pltpu.roll(er, 1, 0))
                hi = jnp.where(row == 0, in_i, pltpu.roll(ei, 1, 0))
                in_r = jnp.broadcast_to(er[7:8], (8, 128))
                in_i = jnp.broadcast_to(ei[7:8], (8, 128))
                before(hr, slack)
                yield
                hr, hi = after(hr), after(hi)
                for j in range(CH):
                    hr, hi = step(m, c, j, ar, ai, hr, hi)
                    h_s[state_row(slot, 0, m, c), pl.ds(j, 8, stride=CS), :] = kr * hr - ki * hi
                    h_s[state_row(slot, 1, m, c), pl.ds(j, 8, stride=CS), :] = kr * hi + ki * hr
                before(hr, slack)
                yield
            carry_s[0, c] = in_r
            carry_s[1, c] = in_i
    n_scan = 20

    def out_product(acc, names, rounds, load, subtract, rows):
        scheme = GROUPS[names[0]][0]
        for rnd in rounds:
            halves = []
            for i, name in enumerate(names):
                sums = _signed_sums([scheme[r][0] for r in rnd], lambda mk: load(i, *mk))
                halves.append([(sign * w_sign[W_BASE[name] + r],
                                product(gate(v, rows // 8).astype(bf16), name, r))
                               for r, (sign, v) in zip(rnd, sums)])
                yield from results(halves[-1], rows)
            assert all(a[0] == b[0] for a, b in zip(*halves))
            _accumulate(acc, [scheme[r][2] for r in rnd],
                        [(a[0], a[1] - b[1] if subtract else a[1] + b[1]) for a, b in zip(*halves)])

    def stage_c(slot):
        for r0 in range(0, R, RS):
            def load(part, m, c):
                return jnp.concatenate([h_s[state_row(slot, part, m, c), pl.ds(k * CS, CH), :]
                                        for k in range(r0 // CH, (r0 + RS) // CH)], axis=0)
            acc = {}
            yield from out_product(acc, ("cre", "cim"), K5_ROUNDS, load, True, RS)
            for (m, q), v in _finish(acc).items():
                y_s[slot, m, q, pl.ds(r0, RS), :] = v
    n_c = 2 * n_group

    def stage_down(slot, lo, hi, rows):
        for r0 in range(lo, hi, rows):
            def load(group, m, k):
                return a_s[slot, group * 7 + k, m, pl.ds(r0, rows), :]
            acc = {}
            yield from out_product(acc, ("dA", "dB"), K7_ROUNDS[:7], load, False, rows)
            for m in range(2):
                done = [acc.pop((m, k)) for k in K7_FOLD]
                _accumulate(acc, [{(m, q + 1): sign for q, sign in fold.items()} for fold in K7_FOLD.values()], done)
            yield from out_product(acc, ("dA", "dB"), K7_ROUNDS[7:], load, False, rows)
            for (m, q), v in _finish(acc).items():
                z_s[m, q - 1, pl.ds(r0, rows), :] = v
    n_down = (R // 8) * 2 * len(K7_ROUNDS)

    def out_copy(b, slot, lo=0, rows=R, k=0):
        return pltpu.make_async_copy(o_s.at[slot, :, pl.ds(lo, rows)], o_hbm.at[b, :, pl.ds(lo, rows)],
                                     out_sem.at[slot, k])

    def stage_out(b, stat_slot, out_slot, slot, lo=0, hi=R):
        row0 = first_row(b)
        for i in range(lo, hi, 16):
            for m in range(2):
                x16 = x_s[pl.ds(row0 + m * R + i, 16), :].astype(f32)
                mu = st_s[stat_slot * 2, pl.ds(m * R + i, 16), :]
                rstd = st_s[stat_slot * 2 + 1, pl.ds(m * R + i, 16), :]
                for c in range(5):
                    x = x16[:, c * 128:(c + 1) * 128]
                    skip = jnp.concatenate([after(par_s[10, c])] * 2, axis=0)
                    hz = z_s[m, c, pl.ds(i, 16), :] * 0.25
                    s = y_s[slot, m, c, pl.ds(i, 16), :] + ((x - mu) * rstd) * skip
                    o_s[out_slot, m, pl.ds(i, 16), pl.ds(c * 128, 128)] = x + s * (hz + hz * jnp.tanh(hz))
                    yield
    n_out = (R // 16) * 10

    def finish_block(b, slot, send, norm=None):
        for r0 in range(0, R, RT):
            fg = stage_down(slot, r0, r0 + RT, RT)
            if norm is not None and r0 < 2 * RT:
                fg = _merge(fg, n_down * RT // R, _take(norm, 10), 10)
            if r0:
                fg = _merge(fg, n_down * RT // R, stage_out(b, b % 3, b % 2, slot, r0 - RT, r0), n_out * RT // R, 0.5)
            _drain(fg)
            if r0 and send:
                out_copy(b, b % 2, r0 - RT, RT, r0 // RT - 1).start()
        if norm is not None:
            _drain(norm)
        reset()
        _drain(stage_out(b, b % 3, b % 2, slot, R - RT, R))
        if send:
            out_copy(b, b % 2, R - RT, RT, R // RT - 1).start()
            for r0 in range(0, R, RT):
                out_copy(b, b % 2, r0, RT, r0 // RT).wait()

    def both(fg0, fg1, n_fg, bg, n_bg, upto):
        _drain(_merge(fg0, n_fg, _take(bg, n_bg // 2), n_bg // 2, upto))
        _drain(_merge(fg1, n_fg, bg, n_bg - n_bg // 2, upto))

    def ahead(fg, steps, *names):
        _drain(_take(fg, steps))
        for name in names:
            copy[name].wait()
        return fg, n_group - steps

    def with_scan(fg, scan):
        return _merge(fg, n_group, _take(scan, n_scan // 2), n_scan // 2, 0.95)

    s0, s1 = 1, 0
    scan0, scan1 = stage_scan(s0, 220), stage_scan(s1, 220)
    ssm_params()
    x_copy[0].wait()
    norm_and_sums(0, s0)
    x_copy[1].wait()
    norm_and_sums(1, s1)
    wait("gl", "ul")
    _drain(prepare("l"))
    _drain(_chain(stage_last(s0), stage_last(s1)))
    wait("bre")
    _drain(prepare("bre"))
    _drain(stage_b(s0, 0))
    _drain(_merge(*ahead(stage_b(s1, 0), R // 8, "bim"), *prepares("bim"), 0.75))
    _drain(stage_b(s0, 1))
    _drain(_merge(*ahead(stage_b(s1, 1), R // 4, "gA", "uA"), *prepares("gA"), 0.75))
    g0, g1 = {}, {}
    both(with_scan(in_product(g0, s0, "gA"), scan0), with_scan(in_product(g1, s1, "gA"), scan0),
         n_group, *prepares("uA"), 0.75)
    _drain(stage_up(g0, s0, 0))
    wait("gB", "uB", "gm", "um")
    _drain(_merge(stage_up(g1, s1, 0), n_group, *prepares("gB"), 0.8))
    _drain(scan0)
    g0, g1 = {}, {}
    both(with_scan(in_product(g0, s0, "gB"), scan1), with_scan(in_product(g1, s1, "gB"), scan1),
         n_group, *prepares("uB"), 0.75)
    both(stage_up(g0, s0, 1), stage_up(g1, s1, 1), n_group, *prepares("m"), 0.7)
    _drain(scan1)
    wait("cre", "cim", "dA")
    both(stage_mixed(s0), stage_mixed(s1), n_group, *prepares("cre", "cim"), 0.7)
    _drain(_merge(stage_c(s0), n_c, *prepares("dA")))
    wait("dB")
    x_copy[2].wait()
    norm2 = stage_norm(2, 2)
    _drain(_merge(_merge(stage_c(s1), n_c, _take(norm2, 12), 12, 1.0, 0.3), n_c, *prepares("dB")))
    finish_block(0, s0, False, norm2)
    out_copy(0, 0).start()
    for cp in x_copy[3:]:
        cp.wait()

    def body(b, carry):
        reset()
        slot = lax.rem(b, 2)
        _drain(_merge(stage_down(0, 0, R, RS), n_down, stage_sums(), n_sums, 0.85))
        fg = _merge(_chain(stage_b(0, 0), stage_b(0, 1)), 2 * n_group,
                    stage_out(b - 1, lax.rem(b - 1, 3), 1 - slot, 0), n_out)
        norm = stage_norm(jnp.minimum(b + 1, NB - 1), lax.rem(b + 1, 3))
        _drain(_merge(fg, 2 * n_group, _take(norm, n_norm // 2), n_norm // 2))
        out_copy(b - 1, 1 - slot).start()
        fg = _chain(stage_ffn(0, 0), stage_ffn(0, 1), stage_mixed(0), stage_last(0))
        _drain(_merge(_merge(fg, n_ffn, norm, n_norm // 2, 0.3), n_ffn, stage_scan(0, 160), n_scan, 0.92))
        _drain(stage_c(0))
        out_copy(b - 2, slot).wait()
        return carry

    lax.fori_loop(2, NB, body, 0)
    reset()
    finish_block(NB - 1, 0, True)
    out_copy(NB - 2, NB % 2).wait()


@jax.jit
def pallas_recurrent_scan__ssm_conv_s5__geglu_ffn__prompt_kernel(
    A_x: jax.Array,
    A_Lambda_re: jax.Array,
    A_Lambda_im: jax.Array,
    A_B_re: jax.Array,
    A_B_im: jax.Array,
    A_C_re: jax.Array,
    A_C_im: jax.Array,
    A_log_dt: jax.Array,
    A_Dskip: jax.Array,
    B_x: jax.Array,
    B_w_gate: jax.Array,
    B_w_up: jax.Array,
    B_w_down: jax.Array,
):
    del B_x
    hbm = pl.BlockSpec(memory_space=pltpu.HBM)
    vmem = pltpu.VMEM
    out = pl.pallas_call(
        _kernel,
        in_specs=[hbm] * 12,
        out_specs=hbm,
        out_shape=jax.ShapeDtypeStruct((NB, 2, R, D), f32),
        scratch_shapes=[
            vmem((L, D), bf16),
            vmem((P, D), bf16), vmem((P, D), bf16),
            vmem((D, P), bf16), vmem((D, P), bf16),
            vmem((F, D), bf16), vmem((F, D), bf16), vmem((F, D), bf16),
            vmem((NW, 128, 128), bf16),
            vmem((2, len(K5), R, 128), bf16),
            vmem((6, T, 128), f32),
            vmem((5, T, 128), f32),
            vmem((11, 5, 8, 128), f32),
            vmem((2, 5, 8, 128), f32),
            vmem((40, HR, 128), f32), vmem((40, HR, 128), f32),
            vmem((2, 14, 2, R, 128), f32),
            vmem((2, 2, 5, R, 128), f32),
            vmem((2, 5, R, 128), f32),
            vmem((2, 2, R, D), f32),
            vmem((P,), bf16), vmem((P,), bf16), vmem((P,), bf16), vmem((D,), bf16),
            pltpu.SemaphoreType.DMA((NB + 18,)),
            pltpu.SemaphoreType.DMA((2, R // RT)),
            pltpu.SemaphoreType.REGULAR(()),
        ],
        compiler_params=pltpu.CompilerParams(vmem_limit_bytes=100 * 1024 * 1024),
    )(A_x.reshape(L, D), A_Lambda_re, A_Lambda_im, A_B_re, A_B_im, A_C_re, A_C_im,
      A_log_dt, A_Dskip, B_w_gate.T, B_w_up.T, B_w_down)
    return out.reshape(1, L, D)
```
